```python
import os as _os
_os.environ.setdefault("JAX_PLATFORMS", "cpu")
import jax
import jax.numpy as jnp

def _softmax(x, axis=-1):
    return jax.nn.softmax(x, axis=axis)
def _gelu(x):
    return jax.nn.gelu(x, approximate=True)
def _silu(x):
    return jax.nn.silu(x)
def _sigmoid(x):
    return jax.nn.sigmoid(x)
def _layernorm(x, axis=-1, eps=1e-5):
    m = jnp.mean(x, axis=axis, keepdims=True)
    v = jnp.var(x, axis=axis, keepdims=True)
    return (x - m) / jnp.sqrt(v + eps)
def _scatter_add(tgt, idx, src, axis=0):
    return tgt.at[idx].add(src)
def _segment_sum(src, seg, n):
    return jax.ops.segment_sum(src, seg, n)
class _Rng:
    def __init__(self, key):
        self._k = key
    def _next(self):
        self._k, sub = jax.random.split(self._k)
        return sub
    def normal(self, shape):
        return jax.random.normal(self._next(), shape, dtype=jnp.bfloat16)
    def randint(self, lo, hi, shape):
        return jax.random.randint(self._next(), shape, lo, hi, dtype=jnp.int32)
    def uniform(self, shape, lo=0.0, hi=1.0):
        return jax.random.uniform(self._next(), shape, jnp.bfloat16, lo, hi)
    def permutation(self, n):
        return jax.random.permutation(self._next(), n)


kernel_name = 'parallel_sum__softmax_full_mha__moe_arch_mod__prompt'

def setup_inputs():
    _rng = _Rng(jax.random.key(int.from_bytes(__import__("os").urandom(4), "little")))
    _w = (lambda a: (lambda t: t.astype(jnp.bfloat16) if jnp.issubdtype(t.dtype, jnp.floating) else t)(jnp.asarray(a)))
    def _A_setup():
        B, S, D = 1, 2048, 512
        return {
            "x": _w((lambda *s: _rng.normal(s) * 0.05)(B, S, D)),
            "wqkv": _w((lambda *s: _rng.normal(s) * 0.1)(D, 3 * D)),
            "wo": _w((lambda *s: _rng.normal(s) * 0.05)(D, D)),
        }
    _A_in = _A_setup()

    def _B_setup():
        B, S, D, F, C = 1, 2048, 512, 1792, 1
        return {
            "x": _w((lambda *s: _rng.normal(s) * 0.05)(B, S, D)),
            "w_r": _w((lambda *s: _rng.normal(s) * 1.6)(D)),
            "w_gate": _w((lambda *s: _rng.normal(s) * 0.1)(D, F)),
            "w_up": _w((lambda *s: _rng.normal(s) * 0.1)(D, F)),
            "w_down": _w((lambda *s: _rng.normal(s) * 0.1)(F, D)),
        }
    _B_in = _B_setup()

    return {
        "A_x": _A_in["x"],
        "A_wqkv": _A_in["wqkv"],
        "A_wo": _A_in["wo"],
        "B_x": _B_in["x"],
        "B_w_r": _B_in["w_r"],
        "B_w_gate": _B_in["w_gate"],
        "B_w_up": _B_in["w_up"],
        "B_w_down": _B_in["w_down"],
    }

def reference(A_x, A_wqkv, A_wo, B_x, B_w_r, B_w_gate, B_w_up, B_w_down):
    def _A_ref(x, wqkv, wo):
        B, S, D = x.shape
        H = 32; Dh = D // H
        qkv = (lambda x, *d: x.transpose(*d))((x @ wqkv).reshape(B, S, 3, H, Dh), 2, 0, 3, 1, 4)
        q, k, v = qkv[0], qkv[1], qkv[2]
        scale = Dh ** -0.5
        scores = jnp.einsum("bhqd,bhkd->bhqk", q, k) * scale
        p = _softmax(scores, axis=-1)
        o = jnp.einsum("bhqk,bhkd->bhqd", p, v)
        return (lambda x, *d: x.transpose(*d))(o, 0, 2, 1, 3).reshape(B, S, D) @ wo

    def _B_ref(x, w_r, w_gate, w_up, w_down):
        B, S, D = x.shape
        C = 1
        r = x @ w_r
        idx = jnp.argsort(-r, axis=-1)[:, :C]
        idx_e = jnp.repeat(idx.reshape(B, C, 1), D, axis=2)
        x_sel = jnp.take_along_axis(x, idx_e, axis=1)
        g = _silu(x_sel @ w_gate)
        u = x_sel @ w_up
        y = (g * u) @ w_down
        r_sel = _sigmoid(jnp.take_along_axis(r, idx, axis=1))
        y = y * r_sel.reshape(B, C, 1)
        b_off = (jnp.arange(B) * S).reshape(B, 1)
        flat_idx = (idx + b_off).reshape(B * C)
        zero = (x * 0.0).reshape(B * S, D)
        upd = _scatter_add(zero, flat_idx, y.reshape(B * C, D), axis=0)
        return x + upd.reshape(B, S, D)

    x = A_x
    xn = _layernorm(x, axis=-1)
    return x + _A_ref(xn, A_wqkv, A_wo) + _B_ref(xn, B_w_r, B_w_gate, B_w_up, B_w_down)
```

```python
import math

import jax
import jax.numpy as jnp
from jax import lax
import jax.experimental.pallas as pl
import jax.experimental.pallas.tpu as pltpu

S = 2048
D = 512
H = 32
DH = 16
F = 1792
TQ = 512
TK = 128
NQ = S // TQ
NK = S // TK
NIT = H * NQ
TR = 256
QSCALE = (DH ** -0.5) * math.log2(math.e)
F32 = jnp.float32
BF16 = jnp.bfloat16


def _bf(v):
    return v.astype(BF16).astype(F32)


def _kernel(x_ref, wqkv_ref, wo_ref, wr_ref, wg_hbm, wu_hbm, wd_hbm, out_ref,
            xn_scr, k_scr, qt_scr, vt_scr, r_scr, ot_scr, wt_scr, sb, mr,
            wg_scr, wu_scr, wd_scr, sems):
    cps = [pltpu.make_async_copy(wg_hbm, wg_scr, sems.at[0]),
           pltpu.make_async_copy(wu_hbm, wu_scr, sems.at[1]),
           pltpu.make_async_copy(wd_hbm, wd_scr, sems.at[2])]
    for c in cps:
        c.start()

    wt_scr[0:D, :] = wqkv_ref[:, 0:D].astype(F32).T.astype(BF16)
    wt_scr[D:2 * D, :] = wqkv_ref[:, 2 * D:3 * D].astype(F32).T.astype(BF16)
    wt_scr[2 * D:2 * D + 16, :] = jnp.broadcast_to(wr_ref[...], (16, D))

    eps = 1.0013580322265625e-05

    def proj(i, _):
        rows = pl.ds(pl.multiple_of(i * TR, TR), TR)
        xf = x_ref[rows, :].astype(F32)
        mean = jnp.sum(xf, axis=1, keepdims=True) * (1.0 / D)
        cen = xf - mean
        var = jnp.sum(cen * cen, axis=1, keepdims=True) * (1.0 / D)
        den = _bf(jnp.sqrt(_bf(_bf(var) + eps)))
        xn = (_bf(xf - _bf(mean)) / den).astype(BF16)
        xn_scr[rows, :] = xn
        k_scr[rows, :] = jnp.dot(xn, wqkv_ref[:, D:2 * D],
                                 preferred_element_type=F32).astype(BF16)
        t = lax.dot_general(wt_scr[...], xn, (((1,), (1,)), ((), ())),
                            preferred_element_type=F32)
        qt_scr[:, rows] = (t[0:D] * QSCALE).astype(BF16)
        vt_scr[:, rows] = t[D:2 * D].astype(BF16)
        r_scr[:, rows] = _bf(t[2 * D:2 * D + 8])
        return 0
    lax.fori_loop(0, S // TR, proj, 0)

    row = lax.broadcasted_iota(jnp.int32, (128, TQ), 0)

    def body(it, _):
        it1 = jnp.minimum(it, NIT - 1)
        h1 = it1 // NQ
        j1 = it1 % NQ
        it2 = jnp.clip(it - 1, 0, NIT - 1)
        h2 = it2 // NQ
        j2 = it2 % NQ
        t1 = h1 // 8
        g1 = h1 % 8
        qt = qt_scr[pl.ds(pl.multiple_of(t1 * 128, 128), 128),
                    pl.ds(pl.multiple_of(j1 * TQ, TQ), TQ)]
        qtm = jnp.where((row >= g1 * 16) & (row < g1 * 16 + 16), qt, jnp.zeros_like(qt))
        m2 = jnp.max(mr[...], axis=0, keepdims=True)
        mx = jnp.full((8, TQ), -jnp.inf, F32)
        l = jnp.zeros((8, TQ), F32)
        o = jnp.zeros((16, TQ), F32)
        for kb in range(NK):
            ks = slice(kb * TK, (kb + 1) * TK)
            p = jnp.exp2(sb[ks, :] - m2)
            l = l + jnp.sum(p.reshape(TK // 8, 8, TQ), axis=0)
            kk = k_scr[ks, pl.ds(pl.multiple_of(t1 * 128, 128), 128)]
            s = jnp.dot(kk, qtm, preferred_element_type=F32)
            sb[ks, :] = s
            mx = jnp.maximum(mx, jnp.max(s.reshape(TK // 8, 8, TQ), axis=0))
            vt = vt_scr[pl.ds(pl.multiple_of(h2 * 16, 16), 16), ks]
            o = o + jnp.dot(vt, p.astype(BF16), preferred_element_type=F32)
        mr[...] = mx
        ls = jnp.sum(l, axis=0, keepdims=True)
        ot_scr[pl.ds(pl.multiple_of(h2 * 16, 16), 16),
               pl.ds(pl.multiple_of(j2 * TQ, TQ), TQ)] = o / ls
        return 0

    sb[...] = jnp.zeros((S, TQ), F32)
    mr[...] = jnp.zeros((8, TQ), F32)
    lax.fori_loop(0, NIT + 1, body, 0)

    r = r_scr[0:1, :]
    rmax = jnp.max(r, axis=1, keepdims=True)
    col = lax.broadcasted_iota(jnp.int32, (1, S), 1)
    idx = jnp.min(jnp.where(r == rmax, col, S), axis=1, keepdims=True)
    for c in cps:
        c.wait()
    rid = lax.broadcasted_iota(jnp.int32, (S, 1), 0)
    xsel = jnp.sum(jnp.where(rid == idx, xn_scr[...].astype(F32), 0.0), axis=0, keepdims=True)
    xsel = jnp.broadcast_to(xsel, (16, D)).astype(BF16)
    g = _bf(jnp.dot(xsel, wg_scr[...], preferred_element_type=F32))
    g = _bf(g * jax.nn.sigmoid(g))
    u = _bf(jnp.dot(xsel, wu_scr[...], preferred_element_type=F32))
    hh = (g * u).astype(BF16)
    y = _bf(jnp.dot(hh, wd_scr[...], preferred_element_type=F32))
    y = _bf(y * _bf(jax.nn.sigmoid(rmax)))[0:1, :]

    def outp(i, _):
        rows = pl.ds(pl.multiple_of(i * TR, TR), TR)
        o = ot_scr[:, rows].T.astype(BF16)
        a = jnp.dot(o, wo_ref[...], preferred_element_type=F32)
        rr = lax.broadcasted_iota(jnp.int32, (TR, 1), 0) + i * TR
        upd = jnp.where(rr == idx, y, 0.0)
        res = (x_ref[rows, :].astype(F32) + a) + (xn_scr[rows, :].astype(F32) + upd)
        out_ref[rows, :] = res.astype(out_ref.dtype)
        return 0
    lax.fori_loop(0, S // TR, outp, 0)


@jax.jit
def pallas_parallel_sum__softmax_full_mha__moe_arch_mod__prompt_kernel(
    A_x: jax.Array,
    A_wqkv: jax.Array,
    A_wo: jax.Array,
    B_x: jax.Array,
    B_w_r: jax.Array,
    B_w_gate: jax.Array,
    B_w_up: jax.Array,
    B_w_down: jax.Array,
):
    x = A_x.reshape(S, D)
    wr = B_w_r.reshape(1, D)
    vm = pl.BlockSpec(memory_space=pltpu.VMEM)
    hbm = pl.BlockSpec(memory_space=pl.ANY)
    out = pl.pallas_call(
        _kernel,
        out_shape=jax.ShapeDtypeStruct((S, D), A_x.dtype),
        in_specs=[vm, vm, vm, vm, hbm, hbm, hbm],
        out_specs=vm,
        scratch_shapes=[
            pltpu.VMEM((S, D), BF16),
            pltpu.VMEM((S, D), BF16),
            pltpu.VMEM((D, S), BF16),
            pltpu.VMEM((D, S), BF16),
            pltpu.VMEM((8, S), F32),
            pltpu.VMEM((D, S), F32),
            pltpu.VMEM((2 * D + 16, D), BF16),
            pltpu.VMEM((S, TQ), F32),
            pltpu.VMEM((8, TQ), F32),
            pltpu.VMEM((D, F), BF16),
            pltpu.VMEM((D, F), BF16),
            pltpu.VMEM((F, D), BF16),
            pltpu.SemaphoreType.DMA((3,)),
        ],
        compiler_params=pltpu.CompilerParams(vmem_limit_bytes=100 * 1024 * 1024),
    )(x, A_wqkv, A_wo, wr, B_w_gate, B_w_up, B_w_down)
    return out.reshape(1, S, D)
```

```python
import math

import jax
import jax.numpy as jnp
from jax import lax
import jax.experimental.pallas as pl
import jax.experimental.pallas.tpu as pltpu

S = 2048
D = 512
H = 32
DH = 16
F = 1792
TQ = 512
TK = 128
NQ = S // TQ
NK = S // TK
NIT = H * NQ
U = 4
LAG = 2
TR = 256
NR = S // TR
TC = 128
QSCALE = (DH ** -0.5) * math.log2(math.e)
EPS = 1.0013580322265625e-05
F32 = jnp.float32
BF16 = jnp.bfloat16


def _bf(v):
    return v.astype(BF16).astype(F32)


def _kernel(x_hbm, wqkv_hbm, wo_hbm, wr_ref, wg_hbm, wu_hbm, wd_hbm, out_hbm,
            x_scr, wqkv_scr, wo_scr, out_scr,
            xn_scr, k_scr, qt_scr, vt_scr, r_scr, ot_scr, o_scr, wt_scr,
            wg_scr, wu_scr, wd_scr, sems, xsems, osems, *tile_scr):
    sbs = tile_scr[0:U]
    mrs = tile_scr[U:2 * U]
    qws = tile_scr[2 * U:3 * U]

    def xcp(i):
        return pltpu.make_async_copy(x_hbm.at[pl.ds(i * TR, TR)], x_scr.at[pl.ds(i * TR, TR)], xsems.at[i])

    def ocp(i):
        return pltpu.make_async_copy(out_scr.at[pl.ds(i * TR, TR)], out_hbm.at[pl.ds(i * TR, TR)], osems.at[i])

    cp_wqkv = pltpu.make_async_copy(wqkv_hbm, wqkv_scr, sems.at[3])
    cp_wo = pltpu.make_async_copy(wo_hbm, wo_scr, sems.at[4])
    cps = [pltpu.make_async_copy(wg_hbm, wg_scr, sems.at[0]),
           pltpu.make_async_copy(wu_hbm, wu_scr, sems.at[1]),
           pltpu.make_async_copy(wd_hbm, wd_scr, sems.at[2])]
    xcp(0).start()
    cp_wqkv.start()

    def layernorm(i):
        rows = pl.ds(i * TR, TR)
        xf = x_scr[rows, :].astype(F32)
        mean = jnp.sum(xf, axis=1, keepdims=True) * (1.0 / D)
        cen = xf - mean
        var = jnp.sum(cen * cen, axis=1, keepdims=True) * (1.0 / D)
        den = _bf(jnp.sqrt(_bf(_bf(var) + EPS)))
        xn_scr[rows, :] = (_bf(xf - _bf(mean)) / den).astype(BF16)

    for u in range(U):
        qws[u][...] = jnp.zeros((128, TQ), BF16)
    xcp(0).wait()
    layernorm(0)
    cp_wqkv.wait()
    for i in range(1, NR):
        xcp(i).start()
    wt_scr[0:D, :] = wqkv_scr[:, 0:D].astype(F32).T.astype(BF16)
    wt_scr[D:2 * D, :] = wqkv_scr[:, 2 * D:3 * D].astype(F32).T.astype(BF16)
    wt_scr[2 * D:2 * D + 16, :] = jnp.broadcast_to(wr_ref[...], (16, D))
    for i in range(1, 3):
        xcp(i).wait()

    for i in range(NR):
        rows = pl.ds(i * TR, TR)
        if i == 2:
            for ii in range(3, NR):
                xcp(ii).wait()
            cp_wo.start()
            for c in cps:
                c.start()
        if i + 1 < NR:
            layernorm(i + 1)
        xn = xn_scr[rows, :]
        k_scr[rows, :] = jnp.dot(xn, wqkv_scr[:, D:2 * D],
                                 preferred_element_type=F32).astype(BF16)
        t = lax.dot_general(wt_scr[...], xn, (((1,), (1,)), ((), ())),
                            preferred_element_type=F32)
        qt_scr[:, rows] = (t[0:D] * QSCALE).astype(BF16)
        vt_scr[:, rows] = t[D:2 * D].astype(BF16)
        r_scr[:, rows] = _bf(t[2 * D:2 * D + 8])

    def mo(v, m):
        return v if isinstance(v, int) else pl.multiple_of(v, m)

    def set_qw(it, u):
        h = it & (H - 1)
        j = it >> 5
        g = h & 7
        gp = (g + 8 - U) & 7
        qw = qws[u]
        qw[pl.ds(mo(gp * 16, 16), 16), :] = jnp.zeros((16, TQ), BF16)
        qw[pl.ds(mo(g * 16, 16), 16), :] = qt_scr[pl.ds(mo(h * 16, 16), 16), pl.ds(mo(j * TQ, TQ), TQ)]

    def step(it1, it2, u, hook=None):
        sb, mr, qw = sbs[u], mrs[u], qws[u]
        if it1 is not None:
            t1 = (it1 & (H - 1)) >> 3
            qtm = qw[...]
            mx = jnp.full((8, TQ), -jnp.inf, F32)
        if it2 is not None:
            h2 = it2 & (H - 1)
            j2 = it2 >> 5
            m2 = jnp.broadcast_to(jnp.max(mr[...], axis=0, keepdims=True), (8, TQ))
            l = jnp.zeros((8, TQ), F32)
            o = jnp.zeros((16, TQ), F32)
        hist = []
        for kb in range(NK):
            ks = slice(kb * TK, (kb + 1) * TK)
            if it2 is not None:
                m2k = m2
                if kb >= LAG:
                    m2k = m2 + hist[kb - LAG] * 0.0
                p = jnp.exp2(sb[ks, :].reshape(TK // 8, 8, TQ) - m2k[None])
                for ii in reversed(range(TK // 16)):
                    l = l + (p[2 * ii] + p[2 * ii + 1])
                hist.append(l)
            if it1 is not None:
                kk = k_scr[ks, pl.ds(mo(t1 * 128, 128), 128)]
                s = jnp.dot(kk, qtm, preferred_element_type=F32)
                sb[ks, :] = s
                mx = jnp.maximum(mx, jnp.max(s.reshape(TK // 8, 8, TQ), axis=0))
            if it2 is not None:
                vt = vt_scr[pl.ds(mo(h2 * 16, 16), 16), ks]
                o = o + jnp.dot(vt, p.reshape(TK, TQ).astype(BF16), preferred_element_type=F32)
            if hook is not None:
                hook(kb)
        if it1 is not None:
            mr[...] = mx
        if it2 is not None:
            cols = pl.ds(mo(j2 * TQ, TQ), TQ)
            ot_scr[pl.ds(mo(h2 * 16, 16), 16), cols] = o * (1.0 / jnp.sum(l, axis=0, keepdims=True))

    for u in range(U):
        set_qw(u, u)
    for u in range(U):
        step(u, None, u)
        set_qw(U + u, u)

    def body(i, _):
        for u in range(U):
            it = U * i + u
            step(it, it - U, u)
            set_qw(jnp.minimum(it + U, NIT - U + u), u)
        return 0
    lax.fori_loop(1, NIT // U, body, 0)

    for c in cps:
        c.wait()
    cp_wo.wait()
    r = r_scr[0:1, :]
    rmax = jnp.max(r, axis=1, keepdims=True)
    col = lax.broadcasted_iota(jnp.int32, (1, S), 1)
    idx = jnp.min(jnp.where(r == rmax, col, S - 1), axis=1, keepdims=True)
    idx_s = idx[0, 0]
    base = pl.multiple_of((idx_s >> 4) << 4, 16)
    blk = xn_scr[pl.ds(base, 16), :].astype(F32)
    rid = lax.broadcasted_iota(jnp.int32, (16, 1), 0) + base
    xsel = jnp.sum(jnp.where(rid == idx, blk, 0.0), axis=0, keepdims=True)
    xsel = jnp.broadcast_to(xsel, (16, D)).astype(BF16)
    g = _bf(jnp.dot(xsel, wg_scr[...], preferred_element_type=F32))
    g = _bf(g * jax.nn.sigmoid(g))
    uu = _bf(jnp.dot(xsel, wu_scr[...], preferred_element_type=F32))
    hh = (g * uu).astype(BF16)
    y = _bf(jnp.dot(hh, wd_scr[...], preferred_element_type=F32))
    y = _bf(y * _bf(jax.nn.sigmoid(rmax)))[0:1, :]

    def otr(c):
        rows = pl.ds(c * TC, TC)
        o_scr[rows, :] = ot_scr[:, rows].T.astype(BF16)

    def outp(c, n):
        rows = pl.ds(c * TC, TC)
        cols = pl.ds(n * 128, 128)
        a = jnp.dot(o_scr[rows, :], wo_scr[:, cols], preferred_element_type=F32)
        rr = lax.broadcasted_iota(jnp.int32, (TC, 1), 0) + c * TC
        upd = jnp.where(rr == idx, y[:, n * 128:(n + 1) * 128], 0.0)
        res = (x_scr[rows, cols].astype(F32) + a) + (xn_scr[rows, cols].astype(F32) + upd)
        out_scr[rows, cols] = res.astype(out_scr.dtype)

    n_early = (S - TQ) // TC
    NP = D // 128
    sched = {}
    for pc in range(n_early * NP):
        sched.setdefault((pc * (U * NK - 1)) // (n_early * NP) + 1, []).append(pc)
    otr(0)

    def hook(t):
        for pc in sched.get(t, []):
            c, n = pc // NP, pc % NP
            if n == 0 and c + 1 < n_early:
                otr(c + 1)
            outp(c, n)

    for u in range(U):
        step(None, NIT - U + u, u, hook=lambda kb, u=u: hook(u * NK + kb))
    for i in range((S - TQ) // TR):
        ocp(i).start()
    for c in range(n_early, S // TC):
        otr(c)
    for c in range(n_early, S // TC):
        for n in range(NP):
            outp(c, n)
        if ((c + 1) * TC) % TR == 0:
            ocp(((c + 1) * TC) // TR - 1).start()
    for i in range(NR):
        ocp(i).wait()


@jax.jit
def pallas_parallel_sum__softmax_full_mha__moe_arch_mod__prompt_kernel(
    A_x: jax.Array,
    A_wqkv: jax.Array,
    A_wo: jax.Array,
    B_x: jax.Array,
    B_w_r: jax.Array,
    B_w_gate: jax.Array,
    B_w_up: jax.Array,
    B_w_down: jax.Array,
):
    x = A_x.reshape(S, D)
    wr = B_w_r.reshape(1, D)
    vm = pl.BlockSpec(memory_space=pltpu.VMEM)
    hbm = pl.BlockSpec(memory_space=pl.ANY)
    out = pl.pallas_call(
        _kernel,
        out_shape=jax.ShapeDtypeStruct((S, D), A_x.dtype),
        in_specs=[hbm, hbm, hbm, vm, hbm, hbm, hbm],
        out_specs=hbm,
        scratch_shapes=[
            pltpu.VMEM((S, D), BF16),
            pltpu.VMEM((D, 3 * D), BF16),
            pltpu.VMEM((D, D), BF16),
            pltpu.VMEM((S, D), BF16),
            pltpu.VMEM((S, D), BF16),
            pltpu.VMEM((S, D), BF16),
            pltpu.VMEM((D, S), BF16),
            pltpu.VMEM((D, S), BF16),
            pltpu.VMEM((8, S), F32),
            pltpu.VMEM((D, S), F32),
            pltpu.VMEM((S, D), BF16),
            pltpu.VMEM((2 * D + 16, D), BF16),
            pltpu.VMEM((D, F), BF16),
            pltpu.VMEM((D, F), BF16),
            pltpu.VMEM((F, D), BF16),
            pltpu.SemaphoreType.DMA((5,)),
            pltpu.SemaphoreType.DMA((NR,)),
            pltpu.SemaphoreType.DMA((NR,)),
        ] + [pltpu.VMEM((S, TQ), F32)] * U
          + [pltpu.VMEM((8, TQ), F32)] * U
          + [pltpu.VMEM((128, TQ), BF16)] * U,
        compiler_params=pltpu.CompilerParams(vmem_limit_bytes=100 * 1024 * 1024),
    )(x, A_wqkv, A_wo, wr, B_w_gate, B_w_up, B_w_down)
    return out.reshape(1, S, D)
```

```python
import math

import jax
import jax.numpy as jnp
from jax import lax
import jax.experimental.pallas as pl
import jax.experimental.pallas.tpu as pltpu

S = 2048
D = 512
H = 32
DH = 16
F = 1792
TQ = 512
TK = 128
NQ = S // TQ
NK = S // TK
NIT = H * NQ
U = 4
LAG = 2
LEAD = 1
PVLAG = 1
TR = 256
NR = S // TR
TC = 128
QSCALE = (DH ** -0.5) * math.log2(math.e)
EPS = 1.0013580322265625e-05
F32 = jnp.float32
BF16 = jnp.bfloat16


def _bf(v):
    return v.astype(BF16).astype(F32)


def _kernel(x_hbm, wqkv_hbm, wo_hbm, wr_ref, wg_hbm, wu_hbm, wd_hbm, out_hbm,
            x_scr, wqkv_scr, wo_scr, out_scr,
            xn_scr, k_scr, qt_scr, vt_scr, r_scr, ot_scr, o_scr, wt_scr,
            wg_scr, wu_scr, wd_scr, sems, xsems, osems, *tile_scr):
    sbs = tile_scr[0:U]
    mrs = tile_scr[U:2 * U]
    qws = tile_scr[2 * U:3 * U]

    def xcp(i):
        return pltpu.make_async_copy(x_hbm.at[pl.ds(i * TR, TR)], x_scr.at[pl.ds(i * TR, TR)], xsems.at[i])

    def ocp(i):
        return pltpu.make_async_copy(out_scr.at[pl.ds(i * TR, TR)], out_hbm.at[pl.ds(i * TR, TR)], osems.at[i])

    cp_wk = pltpu.make_async_copy(wqkv_hbm.at[:, pl.ds(D, D)], wqkv_scr.at[:, pl.ds(D, D)], sems.at[3])
    cp_wq = pltpu.make_async_copy(wqkv_hbm.at[:, pl.ds(0, D)], wqkv_scr.at[:, pl.ds(0, D)], sems.at[5])
    cp_wv = pltpu.make_async_copy(wqkv_hbm.at[:, pl.ds(2 * D, D)], wqkv_scr.at[:, pl.ds(2 * D, D)], sems.at[6])
    cp_wo = pltpu.make_async_copy(wo_hbm, wo_scr, sems.at[4])
    cps = [pltpu.make_async_copy(wg_hbm, wg_scr, sems.at[0]),
           pltpu.make_async_copy(wu_hbm, wu_scr, sems.at[1]),
           pltpu.make_async_copy(wd_hbm, wd_scr, sems.at[2])]
    xcp(0).start()
    cp_wk.start()
    xcp(1).start()

    def layernorm(i):
        rows = pl.ds(i * TR, TR)
        xf = x_scr[rows, :].astype(F32)
        mean = jnp.sum(xf, axis=1, keepdims=True) * (1.0 / D)
        cen = xf - mean
        var = jnp.sum(cen * cen, axis=1, keepdims=True) * (1.0 / D)
        den = _bf(jnp.sqrt(_bf(_bf(var) + EPS)))
        xn_scr[rows, :] = (_bf(xf - _bf(mean)) * (1.0 / den)).astype(BF16)

    def kproj(i):
        rows = pl.ds(i * TR, TR)
        k_scr[rows, :] = jnp.dot(xn_scr[rows, :], wqkv_scr[:, D:2 * D],
                                 preferred_element_type=F32).astype(BF16)

    for u in range(U):
        qws[u][...] = jnp.zeros((128, TQ), BF16)
    xcp(0).wait()
    for i in range(2, NR):
        xcp(i).start()
    cp_wq.start()
    cp_wv.start()
    layernorm(0)
    cp_wk.wait()
    xcp(1).wait()
    layernorm(1)
    kproj(0)
    for i in range(2, 5):
        xcp(i).wait()
    for i in range(1, 4):
        layernorm(i + 1)
        kproj(i)
    for i in range(5, NR):
        xcp(i).wait()
    cp_wq.wait()
    cp_wv.wait()
    cp_wo.start()
    for c in cps:
        c.start()
    wt_scr[0:D, :] = wqkv_scr[:, 0:D].astype(F32).T.astype(BF16)
    wt_scr[D:2 * D, :] = wqkv_scr[:, 2 * D:3 * D].astype(F32).T.astype(BF16)
    wt_scr[2 * D:2 * D + 16, :] = jnp.broadcast_to(wr_ref[...].astype(F32).reshape(1, D), (16, D)).astype(BF16)
    for i in range(4, NR):
        if i + 1 < NR:
            layernorm(i + 1)
        kproj(i)
    for i in range(NR):
        rows = pl.ds(i * TR, TR)
        t = lax.dot_general(wt_scr[...], xn_scr[rows, :], (((1,), (1,)), ((), ())),
                            preferred_element_type=F32)
        qt_scr[:, rows] = (t[0:D] * QSCALE).astype(BF16)
        vt_scr[:, rows] = t[D:2 * D].astype(BF16)
        r_scr[:, rows] = _bf(t[2 * D:2 * D + 8])

    def mo(v, m):
        return v if isinstance(v, int) else pl.multiple_of(v, m)

    def set_qw(it, u):
        h = it & (H - 1)
        j = it >> 5
        g = h & 7
        gp = (g + 8 - U) & 7
        qw = qws[u]
        qw[pl.ds(mo(gp * 16, 16), 16), :] = jnp.zeros((16, TQ), BF16)
        qw[pl.ds(mo(g * 16, 16), 16), :] = qt_scr[pl.ds(mo(h * 16, 16), 16), pl.ds(mo(j * TQ, TQ), TQ)]

    def steps(its1, its2, hook=None, post=None):
        st = [dict() for _ in range(U)]

        def p2(n):
            u, kb = divmod(n, NK)
            d = st[u]
            if kb == 0:
                d['m2'] = jnp.broadcast_to(jnp.max(mrs[u][...], axis=0, keepdims=True), (8, TQ))
                d['l'] = jnp.zeros((8, TQ), F32)
                d['hist'] = []
                d['p'] = {}
            m2k = d['m2']
            if kb >= LAG:
                m2k = m2k + d['hist'][kb - LAG] * 0.0
            p = jnp.exp2(sbs[u][kb * TK:(kb + 1) * TK, :].reshape(TK // 8, 8, TQ) - m2k[None])
            l = d['l']
            for ii in reversed(range(TK // 16)):
                l = l + (p[2 * ii] + p[2 * ii + 1])
            d['l'] = l
            d['hist'].append(l)
            d['p'][kb] = p.reshape(TK, TQ).astype(BF16)

        if its2 is not None:
            for n in range(LEAD):
                p2(n)
        def s1(n):
            u, kb = divmod(n, NK)
            d = st[u]
            ks = slice(kb * TK, (kb + 1) * TK)
            if kb == 0:
                d['qtm'] = qws[u][...]
                d['mx'] = jnp.full((8, TQ), -jnp.inf, F32)
            t1 = (its1[u] & (H - 1)) >> 3
            kk = k_scr[ks, pl.ds(mo(t1 * 128, 128), 128)]
            s = jnp.dot(kk, d['qtm'], preferred_element_type=F32)
            sbs[u][ks, :] = s
            d['mx'] = jnp.maximum(d['mx'], jnp.max(s.reshape(TK // 8, 8, TQ), axis=0))
            if kb == NK - 1:
                mrs[u][...] = d['mx']
                if post is not None:
                    post(u)

        def pv(n):
            u, kb = divmod(n, NK)
            d = st[u]
            ks = slice(kb * TK, (kb + 1) * TK)
            h2 = its2[u] & (H - 1)
            vt = vt_scr[pl.ds(mo(h2 * 16, 16), 16), ks]
            r_ = jnp.dot(vt, d['p'].pop(kb), preferred_element_type=F32)
            d['o'] = r_ if kb == 0 else d['o'] + r_
            if kb == NK - 1:
                j2 = its2[u] >> 5
                ot_scr[pl.ds(mo(h2 * 16, 16), 16), pl.ds(mo(j2 * TQ, TQ), TQ)] = (
                    d['o'] * (1.0 / jnp.sum(d['l'], axis=0, keepdims=True)))

        for n in range(U * NK + PVLAG):
            if its2 is not None and n + LEAD < U * NK:
                p2(n + LEAD)
            if its1 is not None and n < U * NK:
                s1(n)
            if its2 is not None and n >= PVLAG:
                pv(n - PVLAG)
            if hook is not None and n < U * NK:
                hook(n)

    for u in range(U):
        set_qw(u, u)
    steps(list(range(U)), None, post=lambda u: set_qw(U + u, u))

    def body(i, _):
        its = [U * i + u for u in range(U)]
        steps(its, [it - U for it in its],
              post=lambda u: set_qw(jnp.minimum(its[u] + U, NIT - U + u), u))
        return 0
    lax.fori_loop(1, NIT // U, body, 0)

    for c in cps:
        c.wait()
    cp_wo.wait()
    r = r_scr[0:1, :]
    rmax = jnp.max(r, axis=1, keepdims=True)
    col = lax.broadcasted_iota(jnp.int32, (1, S), 1)
    idx = jnp.min(jnp.where(r == rmax, col, S - 1), axis=1, keepdims=True)
    idx_s = idx[0, 0]
    base = pl.multiple_of((idx_s >> 4) << 4, 16)
    blk = xn_scr[pl.ds(base, 16), :].astype(F32)
    rid = lax.broadcasted_iota(jnp.int32, (16, 1), 0) + base
    xsel = jnp.sum(jnp.where(rid == idx, blk, 0.0), axis=0, keepdims=True)
    xsel = jnp.broadcast_to(xsel, (16, D)).astype(BF16)
    g = _bf(jnp.dot(xsel, wg_scr[...], preferred_element_type=F32))
    g = _bf(g * jax.nn.sigmoid(g))
    uu = _bf(jnp.dot(xsel, wu_scr[...], preferred_element_type=F32))
    hh = (g * uu).astype(BF16)
    y = _bf(jnp.dot(hh, wd_scr[...], preferred_element_type=F32))
    y = _bf(y * _bf(jax.nn.sigmoid(rmax)))[0:1, :]

    def otr(c):
        rows = pl.ds(c * TC, TC)
        o_scr[rows, :] = ot_scr[:, rows].T.astype(BF16)

    def outp(c, n):
        rows = pl.ds(c * TC, TC)
        cols = pl.ds(n * 128, 128)
        a = jnp.dot(o_scr[rows, :], wo_scr[:, cols], preferred_element_type=F32)
        rr = lax.broadcasted_iota(jnp.int32, (TC, 1), 0) + c * TC
        upd = jnp.where(rr == idx, y[:, n * 128:(n + 1) * 128], 0.0)
        res = (x_scr[rows, cols].astype(F32) + a) + (xn_scr[rows, cols].astype(F32) + upd)
        out_scr[rows, cols] = res.astype(out_scr.dtype)

    n_early = (S - TQ) // TC
    NP = D // 128
    sched = {}
    for pc in range(n_early * NP):
        sched.setdefault((pc * (U * NK - 1)) // (n_early * NP) + 1, []).append(pc)
    otr(0)

    def hook(t):
        for pc in sched.get(t, []):
            c, n = pc // NP, pc % NP
            if n == 0 and c + 1 < n_early:
                otr(c + 1)
            outp(c, n)
            if n == NP - 1 and ((c + 1) * TC) % TR == 0:
                ocp(((c + 1) * TC) // TR - 1).start()

    steps(None, [NIT - U + u for u in range(U)], hook=hook)
    for c in range(n_early, S // TC):
        otr(c)
    for c in range(n_early, S // TC):
        for n in range(NP):
            outp(c, n)
        if ((c + 1) * TC) % TR == 0:
            ocp(((c + 1) * TC) // TR - 1).start()
    for i in range(NR):
        ocp(i).wait()


@jax.jit
def pallas_parallel_sum__softmax_full_mha__moe_arch_mod__prompt_kernel(
    A_x: jax.Array,
    A_wqkv: jax.Array,
    A_wo: jax.Array,
    B_x: jax.Array,
    B_w_r: jax.Array,
    B_w_gate: jax.Array,
    B_w_up: jax.Array,
    B_w_down: jax.Array,
):
    x = A_x.reshape(S, D)
    wr = B_w_r
    vm = pl.BlockSpec(memory_space=pltpu.VMEM)
    hbm = pl.BlockSpec(memory_space=pl.ANY)
    out = pl.pallas_call(
        _kernel,
        out_shape=jax.ShapeDtypeStruct((S, D), A_x.dtype),
        in_specs=[hbm, hbm, hbm, vm, hbm, hbm, hbm],
        out_specs=hbm,
        scratch_shapes=[
            pltpu.VMEM((S, D), BF16),
            pltpu.VMEM((D, 3 * D), BF16),
            pltpu.VMEM((D, D), BF16),
            pltpu.VMEM((S, D), BF16),
            pltpu.VMEM((S, D), BF16),
            pltpu.VMEM((S, D), BF16),
            pltpu.VMEM((D, S), BF16),
            pltpu.VMEM((D, S), BF16),
            pltpu.VMEM((8, S), F32),
            pltpu.VMEM((D, S), F32),
            pltpu.VMEM((S, D), BF16),
            pltpu.VMEM((2 * D + 16, D), BF16),
            pltpu.VMEM((D, F), BF16),
            pltpu.VMEM((D, F), BF16),
            pltpu.VMEM((F, D), BF16),
            pltpu.SemaphoreType.DMA((7,)),
            pltpu.SemaphoreType.DMA((NR,)),
            pltpu.SemaphoreType.DMA((NR,)),
        ] + [pltpu.VMEM((S, TQ), F32)] * U
          + [pltpu.VMEM((8, TQ), F32)] * U
          + [pltpu.VMEM((128, TQ), BF16)] * U,
        compiler_params=pltpu.CompilerParams(vmem_limit_bytes=100 * 1024 * 1024),
    )(x, A_wqkv, A_wo, wr, B_w_gate, B_w_up, B_w_down)
    return out.reshape(1, S, D)
```

```python
import math

import jax
import jax.numpy as jnp
from jax import lax
import jax.experimental.pallas as pl
import jax.experimental.pallas.tpu as pltpu

S = 2048
D = 512
H = 32
DH = 16
F = 1792
TQ = 512
TK = 128
NQ = S // TQ
NK = S // TK
NIT = H * NQ
U = 4
LAG = 2
LEAD = 1
PVLAG = 1
FD = 6
TR = 256
NR = S // TR
TC = 128
QSCALE = (DH ** -0.5) * math.log2(math.e)
EPS = 1.0013580322265625e-05
F32 = jnp.float32
BF16 = jnp.bfloat16


def _bf(v):
    return v.astype(BF16).astype(F32)


def _kernel(x_hbm, wqkv_hbm, wo_hbm, wr_hbm, wg_hbm, wu_hbm, wd_hbm, out_hbm,
            x_scr, wqkv_scr, wo_scr, out_scr, wr_ref,
            xn_scr, k_scr, qt_scr, vt_scr, r_scr, ot_scr, o_scr, wt_scr,
            wg_scr, wu_scr, wd_scr, sems, xsems, osems, *tile_scr):
    sbs = tile_scr[0:U]
    mrs = tile_scr[U:2 * U]
    qws = tile_scr[2 * U:3 * U]

    def xcp(i):
        return pltpu.make_async_copy(x_hbm.at[pl.ds(i * TR, TR)], x_scr.at[pl.ds(i * TR, TR)], xsems.at[i])

    def ocp(i):
        return pltpu.make_async_copy(out_scr.at[pl.ds(i * TR, TR)], out_hbm.at[pl.ds(i * TR, TR)], osems.at[i])

    cp_wk = pltpu.make_async_copy(wqkv_hbm.at[:, pl.ds(D, D)], wqkv_scr.at[:, pl.ds(D, D)], sems.at[3])
    cp_wq = pltpu.make_async_copy(wqkv_hbm.at[:, pl.ds(0, D)], wqkv_scr.at[:, pl.ds(0, D)], sems.at[5])
    cp_wv = pltpu.make_async_copy(wqkv_hbm.at[:, pl.ds(2 * D, D)], wqkv_scr.at[:, pl.ds(2 * D, D)], sems.at[6])
    cp_wo = pltpu.make_async_copy(wo_hbm, wo_scr, sems.at[4])
    cp_wr = pltpu.make_async_copy(wr_hbm, wr_ref, sems.at[7])
    cps = [pltpu.make_async_copy(wg_hbm, wg_scr, sems.at[0]),
           pltpu.make_async_copy(wu_hbm, wu_scr, sems.at[1]),
           pltpu.make_async_copy(wd_hbm, wd_scr, sems.at[2])]
    xcp(0).start()
    cp_wk.start()
    xcp(1).start()

    def layernorm(i):
        rows = pl.ds(i * TR, TR)
        xf = x_scr[rows, :].astype(F32)
        mean = jnp.sum(xf, axis=1, keepdims=True) * (1.0 / D)
        cen = xf - mean
        var = jnp.sum(cen * cen, axis=1, keepdims=True) * (1.0 / D)
        den = _bf(jnp.sqrt(_bf(_bf(var) + EPS)))
        xn_scr[rows, :] = (_bf(xf - _bf(mean)) * (1.0 / den)).astype(BF16)

    def kproj(i):
        rows = pl.ds(i * TR, TR)
        k_scr[rows, :] = jnp.dot(xn_scr[rows, :], wqkv_scr[:, D:2 * D],
                                 preferred_element_type=F32).astype(BF16)

    for u in range(U):
        qws[u][...] = jnp.zeros((128, TQ), BF16)
    xcp(0).wait()
    for i in range(2, NR):
        xcp(i).start()
    cp_wq.start()
    cp_wv.start()
    cp_wr.start()
    layernorm(0)
    cp_wk.wait()
    xcp(1).wait()
    layernorm(1)
    kproj(0)
    for i in range(2, 5):
        xcp(i).wait()
    for i in range(1, 4):
        layernorm(i + 1)
        kproj(i)
    for i in range(5, NR):
        xcp(i).wait()
    cp_wq.wait()
    cp_wv.wait()
    cp_wr.wait()
    cp_wo.start()
    for c in cps:
        c.start()
    wt_scr[0:D, :] = wqkv_scr[:, 0:D].astype(F32).T.astype(BF16)
    wt_scr[D:2 * D, :] = wqkv_scr[:, 2 * D:3 * D].astype(F32).T.astype(BF16)
    wt_scr[2 * D:2 * D + 16, :] = jnp.broadcast_to(wr_ref[...].astype(F32).reshape(1, D), (16, D)).astype(BF16)
    for i in range(4, NR):
        if i + 1 < NR:
            layernorm(i + 1)
        kproj(i)
    for i in range(NR):
        rows = pl.ds(i * TR, TR)
        t = lax.dot_general(wt_scr[...], xn_scr[rows, :], (((1,), (1,)), ((), ())),
                            preferred_element_type=F32)
        qt_scr[:, rows] = (t[0:D] * QSCALE).astype(BF16)
        vt_scr[:, rows] = t[D:2 * D].astype(BF16)
        r_scr[:, rows] = _bf(t[2 * D:2 * D + 8])

    def mo(v, m):
        return v if isinstance(v, int) else pl.multiple_of(v, m)

    def set_qw(it, u):
        h = it & (H - 1)
        j = it >> 5
        g = h & 7
        gp = (g + 8 - U) & 7
        qw = qws[u]
        qw[pl.ds(mo(gp * 16, 16), 16), :] = jnp.zeros((16, TQ), BF16)
        qw[pl.ds(mo(g * 16, 16), 16), :] = qt_scr[pl.ds(mo(h * 16, 16), 16), pl.ds(mo(j * TQ, TQ), TQ)]

    def steps(its1, its2, hook=None, post=None):
        st = [dict() for _ in range(U)]

        def p2(n):
            u, kb = divmod(n, NK)
            d = st[u]
            if kb == 0:
                d['m2'] = jnp.broadcast_to(jnp.max(mrs[u][...], axis=0, keepdims=True), (8, TQ))
                d['l'] = jnp.zeros((8, TQ), F32)
                d['hist'] = []
                d['p'] = {}
            m2k = d['m2']
            if kb >= LAG:
                m2k = m2k + d['hist'][kb - LAG] * 0.0
            p = jnp.exp2(sbs[u][kb * TK:(kb + 1) * TK, :].reshape(TK // 8, 8, TQ) - m2k[None])
            l = d['l']
            for ii in reversed(range(TK // 16)):
                l = l + (p[2 * ii] + p[2 * ii + 1])
            d['l'] = l
            d['hist'].append(l)
            d['p'][kb] = p.reshape(TK, TQ).astype(BF16)

        if its2 is not None:
            for n in range(LEAD):
                p2(n)
        def s1(n):
            u, kb = divmod(n, NK)
            d = st[u]
            ks = slice(kb * TK, (kb + 1) * TK)
            if kb == 0:
                d['qtm'] = qws[u][...]
                d['mx'] = jnp.full((8, TQ), -jnp.inf, F32)
            t1 = (its1[u] & (H - 1)) >> 3
            kk = k_scr[ks, pl.ds(mo(t1 * 128, 128), 128)]
            s = jnp.dot(kk, d['qtm'], preferred_element_type=F32)
            sbs[u][ks, :] = s
            d['mx'] = jnp.maximum(d['mx'], jnp.max(s.reshape(TK // 8, 8, TQ), axis=0))
            if kb == NK - 1:
                mrs[u][...] = d['mx']
                if post is not None:
                    post(u)

        def pv(n):
            u, kb = divmod(n, NK)
            d = st[u]
            ks = slice(kb * TK, (kb + 1) * TK)
            h2 = its2[u] & (H - 1)
            vt = vt_scr[pl.ds(mo(h2 * 16, 16), 16), ks]
            r_ = jnp.dot(vt, d['p'].pop(kb), preferred_element_type=F32)
            d['o'] = r_ if kb == 0 else d['o'] + r_
            if kb == NK - 1:
                j2 = its2[u] >> 5
                ot_scr[pl.ds(mo(h2 * 16, 16), 16), pl.ds(mo(j2 * TQ, TQ), TQ)] = (
                    d['o'] * (1.0 / jnp.sum(d['l'], axis=0, keepdims=True)))

        for n in range(U * NK + PVLAG):
            if its2 is not None and n + LEAD < U * NK:
                p2(n + LEAD)
            if its1 is not None and n < U * NK:
                s1(n)
            if its2 is not None and n >= PVLAG:
                pv(n - PVLAG)
            if hook is not None and n < U * NK:
                hook(n)

    for u in range(U):
        set_qw(u, u)
    steps(list(range(U)), None, post=lambda u: set_qw(U + u, u))

    def body(i, _):
        its = [U * i + u for u in range(U)]
        steps(its, [it - U for it in its],
              post=lambda u: set_qw(jnp.minimum(its[u] + U, NIT - U + u), u))
        return 0
    lax.fori_loop(1, NIT // U, body, 0)

    for c in cps:
        c.wait()
    cp_wo.wait()
    r = r_scr[0:1, :]
    rmax = jnp.max(r, axis=1, keepdims=True)
    col = lax.broadcasted_iota(jnp.int32, (1, S), 1)
    idx = jnp.min(jnp.where(r == rmax, col, S - 1), axis=1, keepdims=True)
    idx_s = idx[0, 0]
    base = pl.multiple_of((idx_s >> 4) << 4, 16)
    blk = xn_scr[pl.ds(base, 16), :].astype(F32)
    rid = lax.broadcasted_iota(jnp.int32, (16, 1), 0) + base
    xsel = jnp.sum(jnp.where(rid == idx, blk, 0.0), axis=0, keepdims=True)
    xsel = jnp.broadcast_to(xsel, (16, D)).astype(BF16)
    NF = F // 128
    ffn = dict(h=[], y=None)

    def ffn_piece(n):
        if n < NF:
            cs = slice(n * 128, (n + 1) * 128)
            g = _bf(jnp.dot(xsel, wg_scr[:, cs], preferred_element_type=F32))
            g = _bf(g * jax.nn.sigmoid(g))
            uu = _bf(jnp.dot(xsel, wu_scr[:, cs], preferred_element_type=F32))
            ffn['h'].append((g * uu).astype(BF16))
        if FD <= n < FD + NF:
            c = n - FD
            t = jnp.dot(ffn['h'][c], wd_scr[c * 128:(c + 1) * 128, :], preferred_element_type=F32)
            ffn['y'] = t if c == 0 else ffn['y'] + t
            if c == NF - 1:
                ffn['y'] = _bf(_bf(ffn['y']) * _bf(jax.nn.sigmoid(rmax)))[0:1, :]

    def otr(c):
        rows = pl.ds(c * TC, TC)
        o_scr[rows, :] = ot_scr[:, rows].T.astype(BF16)

    def outp(c, n):
        rows = pl.ds(c * TC, TC)
        cols = pl.ds(n * 128, 128)
        a = jnp.dot(o_scr[rows, :], wo_scr[:, cols], preferred_element_type=F32)
        rr = lax.broadcasted_iota(jnp.int32, (TC, 1), 0) + c * TC
        upd = jnp.where(rr == idx, ffn['y'][:, n * 128:(n + 1) * 128], 0.0)
        res = (x_scr[rows, cols].astype(F32) + a) + (xn_scr[rows, cols].astype(F32) + upd)
        out_scr[rows, cols] = res.astype(out_scr.dtype)

    n_early = (S - TQ) // TC
    NP = D // 128
    P0 = FD + NF + 1
    done = []

    def piece(pc):
        c, n = pc // NP, pc % NP
        if n == 0 and c + 1 < n_early:
            otr(c + 1)
        outp(c, n)
        done.append(pc)
        if n == NP - 1 and ((c + 1) * TC) % TR == 0:
            ocp(((c + 1) * TC) // TR - 1).start()

    otr(0)

    def hook(t):
        ffn_piece(t)
        if t >= P0 and t - P0 < n_early * NP:
            piece(t - P0)

    steps(None, [NIT - U + u for u in range(U)], hook=hook)
    for pc in range(len(done), n_early * NP):
        piece(pc)
    for c in range(n_early, S // TC):
        otr(c)
    for pc in range(n_early * NP, (S // TC) * NP):
        piece(pc)
    for i in range(NR):
        ocp(i).wait()


@jax.jit
def pallas_parallel_sum__softmax_full_mha__moe_arch_mod__prompt_kernel(
    A_x: jax.Array,
    A_wqkv: jax.Array,
    A_wo: jax.Array,
    B_x: jax.Array,
    B_w_r: jax.Array,
    B_w_gate: jax.Array,
    B_w_up: jax.Array,
    B_w_down: jax.Array,
):
    x = A_x.reshape(S, D)
    hbm = pl.BlockSpec(memory_space=pl.ANY)
    out = pl.pallas_call(
        _kernel,
        out_shape=jax.ShapeDtypeStruct((S, D), A_x.dtype),
        in_specs=[hbm] * 7,
        out_specs=hbm,
        scratch_shapes=[
            pltpu.VMEM((S, D), BF16),
            pltpu.VMEM((D, 3 * D), BF16),
            pltpu.VMEM((D, D), BF16),
            pltpu.VMEM((S, D), BF16),
            pltpu.VMEM((D,), BF16),
            pltpu.VMEM((S, D), BF16),
            pltpu.VMEM((S, D), BF16),
            pltpu.VMEM((D, S), BF16),
            pltpu.VMEM((D, S), BF16),
            pltpu.VMEM((8, S), F32),
            pltpu.VMEM((D, S), F32),
            pltpu.VMEM((S, D), BF16),
            pltpu.VMEM((2 * D + 16, D), BF16),
            pltpu.VMEM((D, F), BF16),
            pltpu.VMEM((D, F), BF16),
            pltpu.VMEM((F, D), BF16),
            pltpu.SemaphoreType.DMA((8,)),
            pltpu.SemaphoreType.DMA((NR,)),
            pltpu.SemaphoreType.DMA((NR,)),
        ] + [pltpu.VMEM((S, TQ), F32)] * U
          + [pltpu.VMEM((8, TQ), F32)] * U
          + [pltpu.VMEM((128, TQ), BF16)] * U,
        compiler_params=pltpu.CompilerParams(vmem_limit_bytes=100 * 1024 * 1024),
    )(x, A_wqkv, A_wo, B_w_r, B_w_gate, B_w_up, B_w_down)
    return out.reshape(1, S, D)
```

```python
import math

import jax
import jax.numpy as jnp
from jax import lax
import jax.experimental.pallas as pl
import jax.experimental.pallas.tpu as pltpu

S = 2048
D = 512
H = 32
DH = 16
F = 1792
TQ = 512
TK = 128
NQ = S // TQ
NK = S // TK
NIT = H * NQ
U = 4
LAG = 2
LEAD = 1
PVLAG = 1
FD = 6
TR = 256
NR = S // TR
TC = 128
QSCALE = (DH ** -0.5) * math.log2(math.e)
EPS = 1.0013580322265625e-05
F32 = jnp.float32
BF16 = jnp.bfloat16


def _bf(v):
    return v.astype(BF16).astype(F32)


def _kernel(x_hbm, wqkv_hbm, wo_hbm, wr_hbm, wg_hbm, wu_hbm, wd_hbm, out_hbm,
            x_scr, wqkv_scr, wo_scr, out_scr, wr_ref,
            xn_scr, k_scr, qt_scr, vt_scr, r_scr, ot_scr, o_scr, wt_scr,
            wg_scr, wu_scr, wd_scr, sems, xsems, osems, *tile_scr):
    sbs = tile_scr[0:U]
    mrs = tile_scr[U:2 * U]
    qws = tile_scr[2 * U:3 * U]

    def xcp(i):
        return pltpu.make_async_copy(x_hbm.at[pl.ds(i * TR, TR)], x_scr.at[pl.ds(i * TR, TR)], xsems.at[i])

    def ocp(i):
        return pltpu.make_async_copy(out_scr.at[pl.ds(i * TR, TR)], out_hbm.at[pl.ds(i * TR, TR)], osems.at[i])

    cp_wk = pltpu.make_async_copy(wqkv_hbm.at[:, pl.ds(D, D)], wqkv_scr.at[:, pl.ds(D, D)], sems.at[3])
    cp_wq = pltpu.make_async_copy(wqkv_hbm.at[:, pl.ds(0, D)], wqkv_scr.at[:, pl.ds(0, D)], sems.at[5])
    cp_wv = pltpu.make_async_copy(wqkv_hbm.at[:, pl.ds(2 * D, D)], wqkv_scr.at[:, pl.ds(2 * D, D)], sems.at[6])
    cp_wo = pltpu.make_async_copy(wo_hbm, wo_scr, sems.at[4])
    cp_wr = pltpu.make_async_copy(wr_hbm, wr_ref, sems.at[7])
    cps = [pltpu.make_async_copy(wg_hbm, wg_scr, sems.at[0]),
           pltpu.make_async_copy(wu_hbm, wu_scr, sems.at[1]),
           pltpu.make_async_copy(wd_hbm, wd_scr, sems.at[2])]
    xcp(0).start()
    cp_wk.start()
    xcp(1).start()

    def layernorm(i):
        rows = pl.ds(i * TR, TR)
        xf = x_scr[rows, :].astype(F32)
        mean = jnp.sum(xf, axis=1, keepdims=True) * (1.0 / D)
        cen = xf - mean
        var = jnp.sum(cen * cen, axis=1, keepdims=True) * (1.0 / D)
        den = _bf(jnp.sqrt(_bf(_bf(var) + EPS)))
        xn_scr[rows, :] = (_bf(xf - _bf(mean)) * (1.0 / den)).astype(BF16)

    def kproj(i, halves=(0, 1)):
        rows = pl.ds(i * TR, TR)
        for hf in halves:
            c0 = hf * (D // 2)
            k_scr[rows, c0:c0 + D // 2] = jnp.dot(xn_scr[rows, :], wqkv_scr[:, D + c0:D + c0 + D // 2],
                                                  preferred_element_type=F32).astype(BF16)

    for u in range(U):
        qws[u][...] = jnp.zeros((128, TQ), BF16)
    xcp(0).wait()
    for i in range(2, NR):
        xcp(i).start()
    cp_wq.start()
    cp_wv.start()
    cp_wr.start()
    layernorm(0)
    cp_wk.wait()
    xcp(1).wait()
    layernorm(1)
    kproj(0)
    kproj(1, (0,))
    for i in range(2, 5):
        xcp(i).wait()
    kproj(1, (1,))
    for i in range(2, 5):
        layernorm(i)
        kproj(i, (0, 1) if i < 4 else (0,))
    for i in range(5, NR):
        xcp(i).wait()
    cp_wq.wait()
    cp_wv.wait()
    cp_wr.wait()
    cp_wo.start()
    for c in cps:
        c.start()
    kproj(4, (1,))
    wt_scr[0:D, :] = wqkv_scr[:, 0:D].astype(F32).T.astype(BF16)
    wt_scr[D:2 * D, :] = wqkv_scr[:, 2 * D:3 * D].astype(F32).T.astype(BF16)
    wt_scr[2 * D:2 * D + 16, :] = jnp.broadcast_to(wr_ref[...].astype(F32).reshape(1, D), (16, D)).astype(BF16)
    for i in range(5, NR):
        layernorm(i)
        kproj(i)
    for i in range(NR):
        rows = pl.ds(i * TR, TR)
        t = lax.dot_general(wt_scr[...], xn_scr[rows, :], (((1,), (1,)), ((), ())),
                            preferred_element_type=F32)
        qt_scr[:, rows] = (t[0:D] * QSCALE).astype(BF16)
        vt_scr[:, rows] = t[D:2 * D].astype(BF16)
        r_scr[:, rows] = _bf(t[2 * D:2 * D + 8])

    def mo(v, m):
        return v if isinstance(v, int) else pl.multiple_of(v, m)

    def set_qw(it, u):
        h = it & (H - 1)
        j = it >> 5
        g = h & 7
        gp = (g + 8 - U) & 7
        qw = qws[u]
        qw[pl.ds(mo(gp * 16, 16), 16), :] = jnp.zeros((16, TQ), BF16)
        qw[pl.ds(mo(g * 16, 16), 16), :] = qt_scr[pl.ds(mo(h * 16, 16), 16), pl.ds(mo(j * TQ, TQ), TQ)]

    def steps(its1, its2, hook=None, post=None):
        st = [dict() for _ in range(U)]

        def p2(n):
            u, kb = divmod(n, NK)
            d = st[u]
            if kb == 0:
                d['m2'] = jnp.broadcast_to(jnp.max(mrs[u][...], axis=0, keepdims=True), (8, TQ))
                d['l'] = jnp.zeros((8, TQ), F32)
                d['hist'] = []
                d['p'] = {}
            m2k = d['m2']
            if kb >= LAG:
                m2k = m2k + d['hist'][kb - LAG] * 0.0
            p = jnp.exp2(sbs[u][kb * TK:(kb + 1) * TK, :].reshape(TK // 8, 8, TQ) - m2k[None])
            l = d['l']
            for ii in reversed(range(TK // 16)):
                l = l + (p[2 * ii] + p[2 * ii + 1])
            d['l'] = l
            d['hist'].append(l)
            d['p'][kb] = p.reshape(TK, TQ).astype(BF16)

        if its2 is not None:
            for n in range(LEAD):
                p2(n)
        def s1(n):
            u, kb = divmod(n, NK)
            d = st[u]
            ks = slice(kb * TK, (kb + 1) * TK)
            if kb == 0:
                d['qtm'] = qws[u][...]
                d['mx'] = jnp.full((8, TQ), -jnp.inf, F32)
            t1 = (its1[u] & (H - 1)) >> 3
            kk = k_scr[ks, pl.ds(mo(t1 * 128, 128), 128)]
            s = jnp.dot(kk, d['qtm'], preferred_element_type=F32)
            sbs[u][ks, :] = s
            d['mx'] = jnp.maximum(d['mx'], jnp.max(s.reshape(TK // 8, 8, TQ), axis=0))
            if kb == NK - 1:
                mrs[u][...] = d['mx']
                if post is not None:
                    post(u)

        def pv(n):
            u, kb = divmod(n, NK)
            d = st[u]
            ks = slice(kb * TK, (kb + 1) * TK)
            h2 = its2[u] & (H - 1)
            vt = vt_scr[pl.ds(mo(h2 * 16, 16), 16), ks]
            r_ = jnp.dot(vt, d['p'].pop(kb), preferred_element_type=F32)
            d['o'] = r_ if kb == 0 else d['o'] + r_
            if kb == NK - 1:
                j2 = its2[u] >> 5
                ot_scr[pl.ds(mo(h2 * 16, 16), 16), pl.ds(mo(j2 * TQ, TQ), TQ)] = (
                    d['o'] * (1.0 / jnp.sum(d['l'], axis=0, keepdims=True)))

        for n in range(U * NK + PVLAG):
            if its2 is not None and n + LEAD < U * NK:
                p2(n + LEAD)
            if its1 is not None and n < U * NK:
                s1(n)
            if its2 is not None and n >= PVLAG:
                pv(n - PVLAG)
            if hook is not None and n < U * NK:
                hook(n)

    for u in range(U):
        set_qw(u, u)
    steps(list(range(U)), None, post=lambda u: set_qw(U + u, u))

    def body(i, _):
        its = [U * i + u for u in range(U)]
        steps(its, [it - U for it in its],
              post=lambda u: set_qw(jnp.minimum(its[u] + U, NIT - U + u), u))
        return 0
    lax.fori_loop(1, NIT // U, body, 0)

    for c in cps:
        c.wait()
    cp_wo.wait()
    r = r_scr[0:1, :]
    rmax = jnp.max(r, axis=1, keepdims=True)
    col = lax.broadcasted_iota(jnp.int32, (1, S), 1)
    idx = jnp.min(jnp.where(r == rmax, col, S - 1), axis=1, keepdims=True)
    idx_s = idx[0, 0]
    base = pl.multiple_of((idx_s >> 4) << 4, 16)
    blk = xn_scr[pl.ds(base, 16), :].astype(F32)
    rid = lax.broadcasted_iota(jnp.int32, (16, 1), 0) + base
    xsel = jnp.sum(jnp.where(rid == idx, blk, 0.0), axis=0, keepdims=True)
    xsel = jnp.broadcast_to(xsel, (16, D)).astype(BF16)
    NF = F // 128
    ffn = dict(h=[], y=None)

    def ffn_piece(n):
        if n < NF:
            cs = slice(n * 128, (n + 1) * 128)
            g = _bf(jnp.dot(xsel, wg_scr[:, cs], preferred_element_type=F32))
            g = _bf(g * jax.nn.sigmoid(g))
            uu = _bf(jnp.dot(xsel, wu_scr[:, cs], preferred_element_type=F32))
            ffn['h'].append((g * uu).astype(BF16))
        if FD <= n < FD + NF:
            c = n - FD
            t = jnp.dot(ffn['h'][c], wd_scr[c * 128:(c + 1) * 128, :], preferred_element_type=F32)
            ffn['y'] = t if c == 0 else ffn['y'] + t
            if c == NF - 1:
                ffn['y'] = _bf(_bf(ffn['y']) * _bf(jax.nn.sigmoid(rmax)))[0:1, :]

    def otr(c):
        rows = pl.ds(c * TC, TC)
        o_scr[rows, :] = ot_scr[:, rows].T.astype(BF16)

    def outp(c, n):
        rows = pl.ds(c * TC, TC)
        cols = pl.ds(n * 128, 128)
        a = jnp.dot(o_scr[rows, :], wo_scr[:, cols], preferred_element_type=F32)
        rr = lax.broadcasted_iota(jnp.int32, (TC, 1), 0) + c * TC
        upd = jnp.where(rr == idx, ffn['y'][:, n * 128:(n + 1) * 128], 0.0)
        res = (x_scr[rows, cols].astype(F32) + a) + (xn_scr[rows, cols].astype(F32) + upd)
        out_scr[rows, cols] = res.astype(out_scr.dtype)

    n_early = (S - TQ) // TC
    NP = D // 128
    P0 = FD + NF + 1
    done = []

    def piece(pc):
        c, n = pc // NP, pc % NP
        if n == 0 and c + 1 < n_early:
            otr(c + 1)
        outp(c, n)
        done.append(pc)
        if n == NP - 1 and ((c + 1) * TC) % TR == 0:
            ocp(((c + 1) * TC) // TR - 1).start()

    otr(0)

    def hook(t):
        ffn_piece(t)
        if t >= P0 and t - P0 < n_early * NP:
            piece(t - P0)

    steps(None, [NIT - U + u for u in range(U)], hook=hook)
    for pc in range(len(done), n_early * NP):
        piece(pc)
    for c in range(n_early, S // TC):
        otr(c)
    for pc in range(n_early * NP, (S // TC) * NP):
        piece(pc)
    for i in range(NR):
        ocp(i).wait()


@jax.jit
def pallas_parallel_sum__softmax_full_mha__moe_arch_mod__prompt_kernel(
    A_x: jax.Array,
    A_wqkv: jax.Array,
    A_wo: jax.Array,
    B_x: jax.Array,
    B_w_r: jax.Array,
    B_w_gate: jax.Array,
    B_w_up: jax.Array,
    B_w_down: jax.Array,
):
    x = A_x.reshape(S, D)
    hbm = pl.BlockSpec(memory_space=pl.ANY)
    out = pl.pallas_call(
        _kernel,
        out_shape=jax.ShapeDtypeStruct((S, D), A_x.dtype),
        in_specs=[hbm] * 7,
        out_specs=hbm,
        scratch_shapes=[
            pltpu.VMEM((S, D), BF16),
            pltpu.VMEM((D, 3 * D), BF16),
            pltpu.VMEM((D, D), BF16),
            pltpu.VMEM((S, D), BF16),
            pltpu.VMEM((D,), BF16),
            pltpu.VMEM((S, D), BF16),
            pltpu.VMEM((S, D), BF16),
            pltpu.VMEM((D, S), BF16),
            pltpu.VMEM((D, S), BF16),
            pltpu.VMEM((8, S), F32),
            pltpu.VMEM((D, S), F32),
            pltpu.VMEM((S, D), BF16),
            pltpu.VMEM((2 * D + 16, D), BF16),
            pltpu.VMEM((D, F), BF16),
            pltpu.VMEM((D, F), BF16),
            pltpu.VMEM((F, D), BF16),
            pltpu.SemaphoreType.DMA((8,)),
            pltpu.SemaphoreType.DMA((NR,)),
            pltpu.SemaphoreType.DMA((NR,)),
        ] + [pltpu.VMEM((S, TQ), F32)] * U
          + [pltpu.VMEM((8, TQ), F32)] * U
          + [pltpu.VMEM((128, TQ), BF16)] * U,
        compiler_params=pltpu.CompilerParams(vmem_limit_bytes=100 * 1024 * 1024),
    )(x, A_wqkv, A_wo, B_w_r, B_w_gate, B_w_up, B_w_down)
    return out.reshape(1, S, D)
```
